```python
import os as _os
_os.environ.setdefault('JAX_PLATFORMS', 'cpu')
import jax
import jax.numpy as jnp

def _softmax(x, axis=-1):
    return jax.nn.softmax(x, axis=axis)

def _gelu(x):
    return jax.nn.gelu(x, approximate=True)

def _silu(x):
    return jax.nn.silu(x)

def _sigmoid(x):
    return jax.nn.sigmoid(x)

def _layernorm(x, axis=-1, eps=1e-05):
    m = jnp.mean(x, axis=axis, keepdims=True)
    v = jnp.var(x, axis=axis, keepdims=True)
    return (x - m) / jnp.sqrt(v + eps)

def _scatter_add(tgt, idx, src, axis=0):
    return tgt.at[idx].add(src)

def _segment_sum(src, seg, n):
    return jax.ops.segment_sum(src, seg, n)

class _Rng:

    def __init__(self, key):
        self._k = key

    def _next(self):
        self._k, sub = jax.random.split(self._k)
        return sub

    def normal(self, shape):
        return jax.random.normal(self._next(), shape, dtype=jnp.bfloat16)

    def randint(self, lo, hi, shape):
        return jax.random.randint(self._next(), shape, lo, hi, dtype=jnp.int32)

    def uniform(self, shape, lo=0.0, hi=1.0):
        return jax.random.uniform(self._next(), shape, jnp.bfloat16, lo, hi)

    def permutation(self, n):
        return jax.random.permutation(self._next(), n)
kernel_name = 'sequential_preLN__linear_attn_block__mixer_gmlp__prompt'

def setup_inputs():
    _rng = _Rng(jax.random.key(int.from_bytes(__import__("os").urandom(4), "little")))
    _w = lambda a: (lambda t: t.astype(jnp.bfloat16) if jnp.issubdtype(t.dtype, jnp.floating) else t)(jnp.asarray(a))

    def _A_setup():
        B, S, D = (1, 2048, 512)
        return {'x': _w((lambda *s: _rng.normal(s) * 0.05)(B, S, D)), 'wqkv': _w((lambda *s: _rng.normal(s) * 0.05)(D, 3 * D)), 'wo': _w((lambda *s: _rng.normal(s) * 0.05)(D, D))}
    _A_in = _A_setup()

    def _B_setup():
        B, S, D, F = (1, 2048, 512, 1792)
        Fh = F // 2
        return {'x': _w((lambda *s: _rng.normal(s) * 0.05)(B, S, D)), 'w_in': _w((lambda *s: _rng.normal(s) * 0.4)(D, 2 * Fh)), 'w_sp': _w(0.01 * (lambda *s: _rng.normal(s) * 0.4)(S, S)), 'b_sp': _w(1.0 + 0.01 * (lambda *s: _rng.normal(s) * 0.05)(S)), 'w_out': _w((lambda *s: _rng.normal(s) * 0.05)(Fh, D))}
    _B_in = _B_setup()
    return {'A_x': _A_in['x'], 'A_wqkv': _A_in['wqkv'], 'A_wo': _A_in['wo'], 'B_x': _B_in['x'], 'B_w_in': _B_in['w_in'], 'B_w_sp': _B_in['w_sp'], 'B_b_sp': _B_in['b_sp'], 'B_w_out': _B_in['w_out']}

def reference(A_x, A_wqkv, A_wo, B_x, B_w_in, B_w_sp, B_b_sp, B_w_out):

    def _A_ref(x, wqkv, wo):
        B, S, D = x.shape
        H = 32
        Dh = D // H
        qkv = (lambda x, *d: x.transpose(*d))((x @ wqkv).reshape(B, S, 3, H, Dh), 2, 0, 3, 1, 4)
        q, k, v = (qkv[0], qkv[1], qkv[2])
        phi = lambda t: jnp.where(t > 0, t + 1, jnp.exp(t)) + 1e-06
        pq, pk = (phi(q), phi(k))
        kv = jnp.einsum('bhsd,bhse->bhde', pk, v)
        z = jnp.einsum('bhsd->bhd', pk)
        num = jnp.einsum('bhqd,bhde->bhqe', pq, kv)
        den = jnp.einsum('bhqd,bhd->bhq', pq, z)[..., None] + 1e-06
        o = num / den
        return (lambda x, *d: x.transpose(*d))(o, 0, 2, 1, 3).reshape(B, S, D) @ wo

    def _B_ref(x, w_in, w_sp, b_sp, w_out):
        B, S, D = x.shape
        F = w_in.shape[-1]
        Fh = F // 2
        z = _gelu(jnp.einsum('bsd,df->bsf', x, w_in))
        z1 = z[..., :Fh].copy()
        z2 = _layernorm(z[..., Fh:], axis=-1)
        g = jnp.einsum('ts,bsf->btf', w_sp, z2) + b_sp[None, :, None]
        return jnp.einsum('bsf,fd->bsd', z1 * g, w_out)
    x = A_x
    h = x + _A_ref(_layernorm(x, axis=-1), A_wqkv, A_wo)
    h2 = h + _B_ref(_layernorm(h, axis=-1), B_w_in, B_w_sp, B_b_sp, B_w_out)
    return h2
```

```python
import math
import jax
import jax.numpy as jnp
from jax import lax
import jax.experimental.pallas as pl
import jax.experimental.pallas.tpu as pltpu

S, D, H, DH, FH = 2048, 512, 32, 16, 896
F32, BF16 = jnp.float32, jnp.bfloat16
T = 256
NT_ = S // T
TD = 512
OB = 128
NB = 1
RB = T // NB
GLUE = "Q00,Q01,G,Q02,Q03,K,Q10,M,Q11,Q12,Q13,a,b".split(",")
UC = 2
ORDER = "O0,O1,O2,O3,Z0,Q0,Q1,Q2,Q3,Z1,Z2,W0,W1,W2,W3,W4,W5,W6,Z3,Z4,Z5,Z6".split(",")


def _dot(a, b):
    return lax.dot_general(a, b, (((1,), (0,)), ((), ())), preferred_element_type=F32)


def _ln(x, eps=1e-5, scale=None):
    n = x.shape[-1]
    m = jnp.sum(x, axis=-1, keepdims=True) * (1.0 / n)
    c = x - m
    v = jnp.sum(c * c, axis=-1, keepdims=True) * (1.0 / n)
    r = lax.rsqrt(v + eps)
    if scale is not None:
        r = r * scale
    return c * r


def _phi(t):
    return jnp.where(t > 0, t + 1.0, jnp.exp(t)) + 1e-6


_C1 = math.sqrt(2.0 / math.pi)
_C2 = _C1 * 0.044715


def _gelu2(x):
    u = x * (_C1 + _C2 * (x * x))
    return x * jnp.tanh(u) + x


def _recip(d):
    return 1.0 / d


def _normq(pq, zrow):
    q = pq.shape[0] // 4
    lane = lax.broadcasted_iota(jnp.int32, (q, 128), 1)

    def xch(v, s):
        return jnp.take_along_axis(v, lane ^ s, axis=1)
    p = pq * zrow
    a, b, c, e = [p[k * q:(k + 1) * q, :] for k in range(4)]
    b3 = (lane & 8) == 0
    b2 = (lane & 4) == 0
    ab = jnp.where(b3, a, b) + xch(jnp.where(b3, b, a), 8)
    cd = jnp.where(b3, c, e) + xch(jnp.where(b3, e, c), 8)
    t = jnp.where(b2, ab, cd) + xch(jnp.where(b2, cd, ab), 4)
    t = t + xch(t, 2)
    t = t + xch(t, 1)
    r = _recip(t + 1e-6)
    outs = []
    for k in range(4):
        idx = (lane & ~15) | ((k & 1) << 3) | ((k >> 1) << 2)
        outs.append(jnp.take_along_axis(r, idx, axis=1))
    return pq * jnp.concatenate(outs, axis=0)


def _kernel(x_hbm, wqkv_hbm, wo_hbm, win_hbm, wsp_hbm, b_hbm, wout_hbm, out_hbm,
            x_v, wqkv_v, wo_v, win_v, wsp_v, b_v, wout_v,
            xn_v, o_v, m_v, z_v, h_v, hn_v, z1_v, z2_v, out_v, bias_v, sems, osems):
    def rows(i):
        if isinstance(i, int):
            return slice(i * T, (i + 1) * T)
        return pl.ds(pl.multiple_of(i * T, T), T)

    def rblk(i, k):
        if isinstance(i, int):
            return slice(i * T + k * RB, i * T + (k + 1) * RB)
        return pl.ds(pl.multiple_of(i * T + k * RB, RB), RB)

    def col(j):
        return slice(j * 128, (j + 1) * 128)

    def cp(src, dst, k):
        return pltpu.make_async_copy(src, dst, sems.at[k])
    c_x0 = cp(x_hbm.at[0:T, :], x_v.at[0:T, :], 0)
    c_x1 = cp(x_hbm.at[T:2 * T, :], x_v.at[T:2 * T, :], 1)
    c_x2 = cp(x_hbm.at[2 * T:, :], x_v.at[2 * T:, :], 2)
    c_wk = cp(wqkv_hbm.at[:, D:2 * D], wqkv_v.at[:, D:2 * D], 3)
    c_wv = cp(wqkv_hbm.at[:, 2 * D:], wqkv_v.at[:, 2 * D:], 4)
    c_wq = cp(wqkv_hbm.at[:, :D], wqkv_v.at[:, :D], 5)
    c_wo = cp(wo_hbm, wo_v, 6)
    c_win = cp(win_hbm, win_v, 7)
    c_wout = cp(wout_hbm, wout_v, 8)
    c_b = cp(b_hbm, b_v, 9)
    c_wsp = cp(wsp_hbm, wsp_v, 10)

    def LNX(i):
        xn_v[rows(i), :] = _ln(x_v[rows(i), :].astype(F32)).astype(BF16)

    def KP(i):
        pk = _phi(_dot(xn_v[rows(i), :], wqkv_v[:, D:2 * D]))
        return pk.astype(BF16).T, jnp.sum(pk.reshape(T // 8, 8, D), axis=0)

    def QP(i, js):
        xn = xn_v[rows(i), :]
        for j in js:
            q = _dot(xn, wqkv_v[:, col(j)])
            o_v[rows(i), col(j)] = _normq(_phi(q), z_v[:, col(j)]).astype(BF16)

    def stage(order, io=None, iq=None, iw=None):
        gs, hs = [None] * 7, [None] * 4
        if io is not None:
            o = o_v[rows(io), :]
        if iw is not None:
            hn = hn_v[rows(iw), :]
        for tok in order:
            k, j = tok[0], int(tok[1])
            if k == 'Q' and iq is not None:
                QP(iq, [j])
            elif k == 'O' and io is not None:
                hs[j] = x_v[rows(io), col(j)].astype(F32) + _dot(o, m_v[:, col(j)])
                h_v[rows(io), col(j)] = hs[j]
            elif k == 'W' and iw is not None:
                gs[j] = _gelu2(_dot(hn, win_v[:, FH + j * 128:FH + (j + 1) * 128]))
            elif k == 'Z' and iw is not None:
                z1_v[rows(iw), col(j)] = _dot(hn, win_v[:, col(j)])
        for b in range(NB):
            if iw is not None:
                z2 = jnp.concatenate([g[b * RB:(b + 1) * RB, :] for g in gs], axis=1)
                z2_v[rblk(iw, b), :] = _ln(z2, 4e-5, 0.5).astype(BF16)
            if io is not None:
                hb = jnp.concatenate([h[b * RB:(b + 1) * RB, :] for h in hs], axis=1)
                hn_v[rblk(io, b), :] = _ln(hb).astype(BF16)

    for c in (c_x0, c_wk, c_x1, c_x2, c_b, c_wq, c_wv, c_wo, c_win, c_wout, c_wsp):
        c.start()

    def GM(i, pkt):
        return _dot(pkt, xn_v[rows(i), :])

    c_x0.wait()
    LNX(0)
    c_wk.wait()
    c_x1.wait()
    pkts = {}
    pkts[0], zacc = KP(0)
    LNX(1)
    pkts[1], zz = KP(1)
    zacc = zacc + zz
    gacc = GM(0, pkts[0])
    c_x2.wait()
    for i in range(2, NT_):
        if i < NT_ - 1:
            gacc = gacc + GM(i - 1, pkts[i - 1])
        LNX(i)
        pkts[i], zz = KP(i)
        zacc = zacc + zz
    gacc = gacc + GM(NT_ - 2, pkts[NT_ - 2])
    z_v[...] = jnp.sum(zacc, axis=0, keepdims=True)
    for c in (c_b, c_wq, c_wv, c_wo):
        c.wait()
    b2 = b_v[...].astype(F32) * 0.5
    for t in range(S // 128):
        bias_v[t * 128:(t + 1) * 128, :] = jnp.broadcast_to(b2[t:t + 1, :], (128, 128)).T

    ri = lax.broadcasted_iota(jnp.int32, (128, 128), 0) // DH
    ci = lax.broadcasted_iota(jnp.int32, (128, 128), 1) // DH
    mask = ri == ci
    st = {}
    def G7():
        st['g'] = (gacc + GM(NT_ - 1, pkts[NT_ - 1])).astype(BF16)
    def KV():
        st['kv'] = []
        for j in range(4):
            kv = _dot(st['g'][col(j), :], wqkv_v[:, 2 * D + j * 128:2 * D + (j + 1) * 128])
            st['kv'].append(jnp.where(mask, kv, 0.0).astype(BF16))
    def MM():
        for j in range(4):
            m_v[col(j), :] = _dot(st['kv'][j], wo_v[col(j), :]).astype(BF16)
    def OH(hh, n=128):
        rr = slice(hh * n, (hh + 1) * n)
        hb = x_v[rr, :].astype(F32) + _dot(o_v[rr, :], m_v[...])
        h_v[rr, :] = hb
        hn_v[rr, :] = _ln(hb).astype(BF16)
    fns = dict(G=G7, K=KV, M=MM, a=lambda: OH(0), b=lambda: OH(1), o=lambda: OH(0, 256))
    for tok in GLUE:
        if tok[0] == 'Q':
            QP(int(tok[1]), [int(tok[2])])
        else:
            fns[tok]()
    c_win.wait()
    c_wout.wait()

    def loop_c(p, _):
        for u in range(UC):
            i = UC * p + 1 + u
            stage(ORDER, io=i, iq=i + 1, iw=i - 1)
        return 0

    lax.fori_loop(0, (NT_ - 2) // UC, loop_c, 0)
    stage(ORDER, io=NT_ - 1, iw=NT_ - 2)
    stage(ORDER, iw=NT_ - 1)
    c_wsp.wait()

    def phase_d(i, _):
        r = pl.ds(pl.multiple_of(i * TD, TD), TD)
        z1 = _gelu2(z1_v[r, :])
        bcol = bias_v[r, :]
        g = _dot(wsp_v[r, :], z2_v[...]) + jnp.concatenate([bcol] * 7, axis=1)
        zg = (z1 * g).astype(BF16)
        for k in range(TD // OB):
            rk = pl.ds(pl.multiple_of(i * TD + k * OB, OB), OB)
            y = _dot(zg[k * OB:(k + 1) * OB, :], wout_v[...])
            out_v[rk, :] = (h_v[rk, :] + y).astype(BF16)
            pltpu.make_async_copy(out_v.at[rk, :], out_hbm.at[rk, :], osems.at[i * (TD // OB) + k]).start()
        return 0

    lax.fori_loop(0, S // TD, phase_d, 0)
    for i in range(S // OB):
        r = pl.ds(i * OB, OB)
        pltpu.make_async_copy(out_v.at[r, :], out_hbm.at[r, :], osems.at[i]).wait()


@jax.jit
def pallas_sequential_preLN__linear_attn_block__mixer_gmlp__prompt_kernel(A_x, A_wqkv, A_wo, B_x, B_w_in, B_w_sp, B_b_sp, B_w_out):
    del B_x
    x = A_x.reshape(S, D)
    b = B_b_sp.reshape(S // 128, 128)
    anyspec = pl.BlockSpec(memory_space=pl.ANY)
    out = pl.pallas_call(
        _kernel,
        out_shape=jax.ShapeDtypeStruct((S, D), BF16),
        in_specs=[anyspec] * 7,
        out_specs=anyspec,
        scratch_shapes=[
            pltpu.VMEM((S, D), BF16), pltpu.VMEM((D, 3 * D), BF16), pltpu.VMEM((D, D), BF16),
            pltpu.VMEM((D, 2 * FH), BF16), pltpu.VMEM((S, S), BF16), pltpu.VMEM((S // 128, 128), BF16),
            pltpu.VMEM((FH, D), BF16),
            pltpu.VMEM((S, D), BF16), pltpu.VMEM((S, D), BF16), pltpu.VMEM((D, D), BF16),
            pltpu.VMEM((1, D), F32), pltpu.VMEM((S, D), F32), pltpu.VMEM((S, D), BF16),
            pltpu.VMEM((S, FH), F32), pltpu.VMEM((S, FH), BF16), pltpu.VMEM((S, D), BF16),
            pltpu.VMEM((S, 128), F32),
            pltpu.SemaphoreType.DMA((11,)), pltpu.SemaphoreType.DMA((S // OB,)),
        ],
        compiler_params=pltpu.CompilerParams(vmem_limit_bytes=100 * 1024 * 1024),
    )(x, A_wqkv, A_wo, B_w_in, B_w_sp, b, B_w_out)
    return out.reshape(1, S, D)
```
